```python
import os as _os
_os.environ.setdefault("JAX_PLATFORMS", "cpu")
import jax
import jax.numpy as jnp

def _softmax(x, axis=-1):
    return jax.nn.softmax(x, axis=axis)
def _gelu(x):
    return jax.nn.gelu(x, approximate=True)
def _silu(x):
    return jax.nn.silu(x)
def _sigmoid(x):
    return jax.nn.sigmoid(x)
def _layernorm(x, axis=-1, eps=1e-5):
    m = jnp.mean(x, axis=axis, keepdims=True)
    v = jnp.var(x, axis=axis, keepdims=True)
    return (x - m) / jnp.sqrt(v + eps)
def _scatter_add(tgt, idx, src, axis=0):
    return tgt.at[idx].add(src)
def _segment_sum(src, seg, n):
    return jax.ops.segment_sum(src, seg, n)
class _Rng:
    def __init__(self, key):
        self._k = key
    def _next(self):
        self._k, sub = jax.random.split(self._k)
        return sub
    def normal(self, shape):
        return jax.random.normal(self._next(), shape, dtype=jnp.bfloat16)
    def randint(self, lo, hi, shape):
        return jax.random.randint(self._next(), shape, lo, hi, dtype=jnp.int32)
    def uniform(self, shape, lo=0.0, hi=1.0):
        return jax.random.uniform(self._next(), shape, jnp.bfloat16, lo, hi)
    def permutation(self, n):
        return jax.random.permutation(self._next(), n)


kernel_name = 'parallel_sum__linear_kernel_hedgehog__dense_activation_gelu__prompt'

def setup_inputs():
    _rng = _Rng(jax.random.key(int.from_bytes(__import__("os").urandom(4), "little")))
    _w = (lambda a: (lambda t: t.astype(jnp.bfloat16) if jnp.issubdtype(t.dtype, jnp.floating) else t)(jnp.asarray(a)))
    def _A_setup():
        B, S, D, H = 1, 2048, 448, 16
        Dh = D // H
        return {
            "x": _w((lambda *s: _rng.normal(s) * 0.05)(B, S, D)),
            "wqkv": _w((lambda *s: _rng.normal(s) * 0.2)(D, 3 * D)),
            "w_phi": _w((lambda *s: _rng.normal(s) * 0.2)(H, Dh, Dh) * (Dh ** -0.5)),
            "wo": _w((lambda *s: _rng.normal(s) * 0.05)(D, D)),
        }
    _A_in = _A_setup()

    def _B_setup():
        B, S, D, F = 1, 2048, 448, 1792
        return {
            "x": _w((lambda *s: _rng.normal(s) * 0.05)(B, S, D)),
            "w1": _w((lambda *s: _rng.normal(s) * 0.2)(D, F) * (D ** -0.5)),
            "b1": _w((lambda *s: _rng.normal(s) * 0.2)(F) * 0.01),
            "w2": _w((lambda *s: _rng.normal(s) * 0.2)(F, D) * (F ** -0.5)),
            "b2": _w((lambda *s: _rng.normal(s) * 0.05)(D) * 0.01),
        }
    _B_in = _B_setup()

    return {
        "A_x": _A_in["x"],
        "A_wqkv": _A_in["wqkv"],
        "A_w_phi": _A_in["w_phi"],
        "A_wo": _A_in["wo"],
        "B_x": _B_in["x"],
        "B_w1": _B_in["w1"],
        "B_b1": _B_in["b1"],
        "B_w2": _B_in["w2"],
        "B_b2": _B_in["b2"],
    }

def reference(A_x, A_wqkv, A_w_phi, A_wo, B_x, B_w1, B_b1, B_w2, B_b2):
    def _A_ref(x, wqkv, w_phi, wo):
        B, S, D = x.shape
        H = 16; Dh = D // H
        qkv = (lambda x, *d: x.transpose(*d))((x @ wqkv).reshape(B, S, 3, H, Dh), 2, 0, 3, 1, 4)
        q, k, v = qkv[0], qkv[1], qkv[2]
        pq = jnp.einsum("bhsd,hdf->bhsf", q, w_phi)
        pk = jnp.einsum("bhsd,hdf->bhsf", k, w_phi)
        phi_q = jnp.concatenate([_softmax(pq, axis=-1), _softmax(-pq, axis=-1)], axis=-1)
        phi_k = jnp.concatenate([_softmax(pk, axis=-1), _softmax(-pk, axis=-1)], axis=-1)
        kv = jnp.einsum("bhsf,bhsd->bhfd", phi_k, v)
        z  = jnp.einsum("bhsf->bhf", phi_k)
        num = jnp.einsum("bhqf,bhfd->bhqd", phi_q, kv)
        den = jnp.einsum("bhqf,bhf->bhq", phi_q, z)[..., None] + 1e-6
        o = num / den
        return (lambda x, *d: x.transpose(*d))(o, 0, 2, 1, 3).reshape(B, S, D) @ wo

    def _B_ref(x, w1, b1, w2, b2):
        h = jnp.einsum("bsd,df->bsf", x, w1) + b1
        h = _gelu(h)
        return jnp.einsum("bsf,fd->bsd", h, w2) + b2

    x = A_x
    xn = _layernorm(x, axis=-1)
    return x + _A_ref(xn, A_wqkv, A_w_phi, A_wo) + _B_ref(xn, B_w1, B_b1, B_w2, B_b2)
```

```python
import jax
import jax.numpy as jnp
from jax import lax
import jax.experimental.pallas as pl
import jax.experimental.pallas.tpu as pltpu

S, D, H, DH, F = 2048, 448, 16, 28, 1792
NG = H // 2
GR = 2 * DH
TS = 512
NTILE = S // TS
DE = D + 16
FC = 1792

_NT = (((1,), (1,)), ((), ()))
_NN = (((1,), (0,)), ((), ()))
_F32 = jnp.float32
_BF16 = jnp.bfloat16


def _dot(a, b, dims):
    return lax.dot_general(a, b, dims, preferred_element_type=_F32)


def _dual_softmax(p):
    ts = p.shape[1]
    p3 = p.reshape(7, 8, ts)
    mx = jnp.max(p3, axis=0)
    mn = jnp.min(p3, axis=0)
    mx = jnp.maximum(mx, pltpu.roll(mx, 4, axis=0))
    mx = jnp.maximum(mx, pltpu.roll(mx, 2, axis=0))
    mn = jnp.minimum(mn, pltpu.roll(mn, 4, axis=0))
    mn = jnp.minimum(mn, pltpu.roll(mn, 2, axis=0))
    ep = jnp.exp(p3 - mx[None])
    en = jnp.exp(mn[None] - p3)
    sp = jnp.sum(ep, axis=0)
    sn = jnp.sum(en, axis=0)
    sp = sp + pltpu.roll(sp, 4, axis=0)
    sp = sp + pltpu.roll(sp, 2, axis=0)
    sn = sn + pltpu.roll(sn, 4, axis=0)
    sn = sn + pltpu.roll(sn, 2, axis=0)
    ep = ep * (1.0 / sp)[None]
    en = en * (1.0 / sn)[None]
    phi = jnp.concatenate([ep, en], axis=0).reshape(2 * GR, ts)
    return phi.astype(_BF16)


def _colsum(a3):
    s = jnp.sum(a3, axis=0)
    s = s + pltpu.roll(s, 4, axis=0)
    s = s + pltpu.roll(s, 2, axis=0)
    return s + pltpu.roll(s, 1, axis=0)


def _layernorm_t(xb):
    ts = xb.shape[1]
    x3 = xb.astype(_F32).reshape(D // 8, 8, ts)
    m = _colsum(x3) * (1.0 / D)
    xc = x3 - m[None]
    v = _colsum(xc * xc) * (1.0 / D)
    return (xc * lax.rsqrt(v + 1e-5)[None]).reshape(D, ts)


def _gelu(x):
    c = 0.7978845608028654
    return 0.5 * x * (1.0 + jnp.tanh(x * (c + (c * 0.044715) * (x * x))))


def _kernel(x_hbm, wqkv_hbm, wphi_hbm, wo_hbm, w1_hbm, b1_hbm, w2T_hbm, b2_hbm,
            out_hbm,
            x_v, wqkv_v, wphi_v, wo_v, w1_v, b1_v, w2T_v, b2_v, out_v,
            xn_v, wT_v, wf2_v, wflat_v, phiq_v, kv_v, kvm_v, woT_v, oT_v,
            xsem, wsem, osem):
    def x_copy(i):
        return pltpu.make_async_copy(
            x_hbm.at[0, :, pl.ds(pl.multiple_of(i * TS, TS), TS)], x_v.at[i], xsem.at[i])

    def out_copy(i):
        return pltpu.make_async_copy(
            out_v.at[i], out_hbm.at[0, :, pl.ds(pl.multiple_of(i * TS, TS), TS)], osem.at[i])

    c_wphi = pltpu.make_async_copy(wphi_hbm, wphi_v, wsem.at[0])
    c_wq = pltpu.make_async_copy(wqkv_hbm.at[:, 0:512], wqkv_v.at[:, 0:512], wsem.at[1])
    c_wk = pltpu.make_async_copy(wqkv_hbm.at[:, 512:896], wqkv_v.at[:, 512:896], wsem.at[7])
    c_wv = pltpu.make_async_copy(wqkv_hbm.at[:, 896:1344], wqkv_v.at[:, 896:1344], wsem.at[8])
    c_wo = pltpu.make_async_copy(wo_hbm, wo_v.at[0:D], wsem.at[2])
    c_w1 = pltpu.make_async_copy(w1_hbm, w1_v.at[0:D], wsem.at[3])
    c_w2 = pltpu.make_async_copy(w2T_hbm, w2T_v, wsem.at[4])
    c_b1 = pltpu.make_async_copy(b1_hbm, b1_v, wsem.at[5])
    c_b2 = pltpu.make_async_copy(b2_hbm, b2_v, wsem.at[6])

    c_wphi.start()
    c_wq.start()
    x_copy(0).start()
    c_wk.start()
    c_wv.start()

    e16 = lax.broadcasted_iota(jnp.int32, (16, TS), 0)
    one_rows = jnp.where(e16 == 0, 1.0, 0.0)

    def ln_tile(j):
        for b in range(TS // 128):
            xn = _layernorm_t(x_v[j, :, 128 * b:128 * (b + 1)])
            xn_v[j, 0:D, 128 * b:128 * (b + 1)] = xn.astype(_BF16)

    for j in range(NTILE):
        xn_v[j, D:DE, :] = one_rows.astype(_BF16)

    wflat_v[...] = jnp.zeros(wflat_v.shape, _F32)
    wf2_v[...] = jnp.zeros(wf2_v.shape, _F32)
    kv_v[...] = jnp.zeros(kv_v.shape, _F32)
    c_wphi.wait()
    wf2_v[:, 0:DH] = wphi_v[...].reshape(D, DH).astype(_F32)
    for h in range(H):
        wflat_v[64 + DH * h:64 + DH * (h + 1), :] = wf2_v[pl.ds(h, DH, stride=H), :]
    wfb = wflat_v[...].astype(_BF16)
    rr = lax.broadcasted_iota(jnp.int32, (2 * GR, 128), 0)
    cc = lax.broadcasted_iota(jnp.int32, (2 * GR, 128), 1)
    fr = jnp.where(rr >= GR, rr - GR, rr) >> 1
    rf = jnp.where(cc == fr, 1.0, 0.0).astype(_BF16)
    uq = _dot(rf, wfb[64:576], _NT)
    uk = _dot(rf, wfb[0:512], _NT)
    def amat(u, c, shift, l0, w):
        row = lax.broadcasted_iota(jnp.int32, (2 * GR, w), 0)
        ln = lax.broadcasted_iota(jnp.int32, (2 * GR, w), 1)
        lo = (jnp.where(row >= GR, 2, 0) + (row & 1)) * DH + (112 * c + shift - l0)
        return jnp.where((ln >= lo) & (ln < lo + DH), u[:, l0:l0 + w], 0.0).astype(_BF16)

    q_win = [(0, 128), (0, 256), (128, 256), (256, 256)]
    k_win = [(0, 256), (128, 256), (256, 256), (384, 128)]
    aq = [amat(uq, c, 0, *q_win[c]) for c in range(4)]
    ak = [amat(uk, c, 64, *k_win[c]) for c in range(4)]
    x_copy(0).wait()
    ln_tile(0)
    c_wq.wait()
    x_copy(1).start()
    for c in range(4):
        l0, w = q_win[c]
        wT_v[112 * c:112 * (c + 1), :] = _dot(aq[c], wqkv_v[:, l0:l0 + w], _NT).astype(_BF16)
    c_wk.wait()
    c_wv.wait()
    for i in range(2, NTILE):
        x_copy(i).start()
    for c in range(4):
        l0, w = k_win[c]
        wT_v[D + 112 * c:D + 112 * (c + 1), :] = _dot(
            ak[c], wqkv_v[:, 384 + l0:384 + l0 + w], _NT).astype(_BF16)
    wT_v[2 * D:3 * D, :] = wqkv_v[:, 2 * D:3 * D].T
    c_b1.start()
    c_b2.start()
    c_wo.start()
    c_w1.start()
    c_w2.start()

    def phase1(i, carry):
        @pl.when(i + 1 < NTILE)
        def _():
            x_copy(i + 1).wait()
        xn = xn_v[i, 0:D, :]
        vT = _dot(wT_v[2 * D:3 * D, :], xn, _NN)
        ln_tile(jnp.minimum(i + 1, NTILE - 1))
        phik = []
        for c in range(4):
            p = _dot(wT_v[D + 112 * c:D + 112 * (c + 1), :], xn, _NN)
            phik.append(_dual_softmax(p[0:GR]))
            phik.append(_dual_softmax(p[GR:2 * GR]))
        ones = jnp.ones((8, TS), _F32)

        def kv(g):
            vext = jnp.concatenate([vT[GR * g:GR * (g + 1)], ones], axis=0).astype(_BF16)
            kv_v[g] += _dot(vext, phik[g], _NT)

        kv_after = {0: [], 1: [0, 1], 2: [2, 3], 3: [4, 5, 6, 7]}
        for c in range(4):
            p = _dot(wT_v[112 * c:112 * (c + 1), :], xn, _NN)
            phiq_v[i, 224 * c:224 * c + 112, :] = _dual_softmax(p[0:GR])
            phiq_v[i, 224 * c + 112:224 * (c + 1), :] = _dual_softmax(p[GR:2 * GR])
            for g in kv_after[c]:
                kv(g)
        return carry

    lax.fori_loop(0, NTILE, phase1, 0)

    r2 = lax.broadcasted_iota(jnp.int32, (64, 2 * GR), 0)
    c2 = lax.broadcasted_iota(jnp.int32, (64, 2 * GR), 1)
    rhead = jnp.where(r2 < GR, (r2 >= DH).astype(jnp.int32), (r2 >= GR + 4).astype(jnp.int32))
    keep = rhead == (c2 & 1)
    c_b1.wait()
    c_b2.wait()
    c_wo.wait()
    c_w1.wait()
    c_w2.wait()
    for g in range(NG):
        kvm_v[g] = jnp.where(keep, kv_v[g], 0.0).astype(_BF16)
    b1 = b1_v[...].astype(_F32).reshape(1, F)
    b2 = b2_v[...].astype(_F32).reshape(1, D)
    wo_v[D:DE, :] = jnp.where(lax.broadcasted_iota(jnp.int32, (16, D), 0) == 0, b2, 0.0).astype(_BF16)
    w1_v[D:DE, :] = jnp.where(lax.broadcasted_iota(jnp.int32, (16, F), 0) == 0, b1, 0.0).astype(_BF16)
    sub = lax.broadcasted_iota(jnp.int32, (8, TS), 0)

    def attn_tile(j):
        oT = []
        for g in range(NG):
            n = _dot(kvm_v[g], phiq_v[j, 112 * g:112 * (g + 1), :], _NN)
            r = 1.0 / (n[GR:GR + 8] + 1e-6)
            rs = pltpu.roll(r, 4, axis=0)
            ra = jnp.where(sub < 4, r, rs)
            rb = jnp.where(sub < 4, rs, r)
            oT.append((n[0:24].reshape(3, 8, TS) * ra[None]).reshape(24, TS))
            oT.append(n[24:32] * r)
            oT.append((n[32:56].reshape(3, 8, TS) * rb[None]).reshape(24, TS))
        oT.append(one_rows)
        oT_v[...] = jnp.concatenate(oT, axis=0).astype(_BF16)

    attn_tile(0)
    woT_v[...] = wo_v[...].T

    def phase2(i, carry):
        acc = _dot(woT_v[...], oT_v[...], _NN) + x_v[i].astype(_F32)
        xnat = xn_v[i].T
        for c in range(F // FC):
            h = _gelu(_dot(xnat, w1_v[:, FC * c:FC * (c + 1)], _NN)).astype(_BF16)
            acc = acc + _dot(w2T_v[:, FC * c:FC * (c + 1)], h, _NT)
        attn_tile(jnp.minimum(i + 1, NTILE - 1))
        out_v[i] = acc.astype(_BF16)
        out_copy(i).start()
        return carry

    lax.fori_loop(0, NTILE, phase2, 0)
    for i in range(NTILE):
        out_copy(i).wait()


@jax.jit
def pallas_parallel_sum__linear_kernel_hedgehog__dense_activation_gelu__prompt_kernel(
    A_x, A_wqkv, A_w_phi, A_wo, B_x, B_w1, B_b1, B_w2, B_b2,
):
    del B_x
    hbm_spec = pl.BlockSpec(memory_space=pltpu.HBM)
    scratch = [
        pltpu.VMEM((NTILE, D, TS), _BF16),
        pltpu.VMEM((D, 3 * D), _BF16),
        pltpu.VMEM((DH, H, DH), _BF16),
        pltpu.VMEM((DE, D), _BF16),
        pltpu.VMEM((DE, F), _BF16),
        pltpu.VMEM((F,), _BF16),
        pltpu.VMEM((D, F), _BF16),
        pltpu.VMEM((D,), _BF16),
        pltpu.VMEM((NTILE, D, TS), _BF16),
        pltpu.VMEM((NTILE, DE, TS), _BF16),
        pltpu.VMEM((3 * D, D), _BF16),
        pltpu.VMEM((D, 128), _F32),
        pltpu.VMEM((576, 128), _F32),
        pltpu.VMEM((NTILE, 2 * D, TS), _BF16),
        pltpu.VMEM((NG, 64, 2 * GR), _F32),
        pltpu.VMEM((NG, 64, 2 * GR), _BF16),
        pltpu.VMEM((D, DE), _BF16),
        pltpu.VMEM((DE, TS), _BF16),
        pltpu.SemaphoreType.DMA((NTILE,)),
        pltpu.SemaphoreType.DMA((9,)),
        pltpu.SemaphoreType.DMA((NTILE,)),
    ]
    outT = pl.pallas_call(
        _kernel,
        in_specs=[hbm_spec] * 8,
        out_specs=hbm_spec,
        out_shape=jax.ShapeDtypeStruct((1, D, S), _BF16),
        scratch_shapes=scratch,
        compiler_params=pltpu.CompilerParams(vmem_limit_bytes=100 * 1024 * 1024),
    )(jnp.transpose(A_x, (0, 2, 1)), A_wqkv, jnp.transpose(A_w_phi, (1, 0, 2)), A_wo,
      B_w1, B_b1, B_w2.T, B_b2)
    return jnp.transpose(outT, (0, 2, 1))
```

```python
import jax
import jax.numpy as jnp
from jax import lax
import jax.experimental.pallas as pl
import jax.experimental.pallas.tpu as pltpu

S, D, H, DH, F = 2048, 448, 16, 28, 1792
NG = H // 2
GR = 2 * DH
TS = 512
NTILE = S // TS
DE = D + 16
NS = 4
HS = TS // NS

_NT = (((1,), (1,)), ((), ()))
_NN = (((1,), (0,)), ((), ()))
_F32 = jnp.float32
_BF16 = jnp.bfloat16


def _dot(a, b, dims):
    return lax.dot_general(a, b, dims, preferred_element_type=_F32)


def _dual_softmax(p):
    ts = p.shape[1]
    p3 = p.reshape(7, 8, ts)
    mx = jnp.max(p3, axis=0)
    mn = jnp.min(p3, axis=0)
    mx = jnp.maximum(mx, pltpu.roll(mx, 4, axis=0))
    mx = jnp.maximum(mx, pltpu.roll(mx, 2, axis=0))
    mn = jnp.minimum(mn, pltpu.roll(mn, 4, axis=0))
    mn = jnp.minimum(mn, pltpu.roll(mn, 2, axis=0))
    ep = jnp.exp(p3 - mx[None])
    en = jnp.exp(mn[None] - p3)
    sp = jnp.sum(ep, axis=0)
    sn = jnp.sum(en, axis=0)
    sp = sp + pltpu.roll(sp, 4, axis=0)
    sp = sp + pltpu.roll(sp, 2, axis=0)
    sn = sn + pltpu.roll(sn, 4, axis=0)
    sn = sn + pltpu.roll(sn, 2, axis=0)
    ep = ep * (1.0 / sp)[None]
    en = en * (1.0 / sn)[None]
    phi = jnp.concatenate([ep, en], axis=0).reshape(2 * GR, ts)
    return phi.astype(_BF16)


def _colsum(a3):
    s = jnp.sum(a3, axis=0)
    s = s + pltpu.roll(s, 4, axis=0)
    s = s + pltpu.roll(s, 2, axis=0)
    return s + pltpu.roll(s, 1, axis=0)


def _layernorm_t(xb):
    n = xb.shape[1]
    x3 = xb.astype(_F32).reshape(D // 8, 8, n)
    m = _colsum(x3) * (1.0 / D)
    xc = x3 - m[None]
    v = _colsum(xc * xc) * (1.0 / D)
    return (xc * lax.rsqrt(v + 1e-5)[None]).reshape(D, n)


def _gelu(x):
    c = 0.7978845608028654
    return 0.5 * x * (1.0 + jnp.tanh(x * (c + (c * 0.044715) * (x * x))))


def _kernel(x_hbm, wqkv_hbm, wphi_hbm, wo_hbm, w1_hbm, b1_hbm, w2T_hbm, b2_hbm,
            out_hbm,
            x_v, wqkv_v, wphi_v, wo_v, w1_v, b1_v, w2T_v, b2_v, out_v,
            xn_v, wT_v, wf2_v, wflat_v, phiq_v, kv_v, kvm_v,
            xsem, wsem, osem):
    def x_copy(i):
        off = i * TS if isinstance(i, int) else pl.multiple_of(i * TS, TS)
        return pltpu.make_async_copy(
            x_hbm.at[0, :, pl.ds(off, TS)], x_v.at[i], xsem.at[i])

    def out_copy(i, p):
        off = i * TS + HS * p
        if not isinstance(i, int):
            off = pl.multiple_of(off, HS)
        return pltpu.make_async_copy(
            out_v.at[i, :, HS * p:HS * (p + 1)],
            out_hbm.at[0, :, pl.ds(off, HS)], osem.at[NS * i + p])

    c_wphi = pltpu.make_async_copy(wphi_hbm, wphi_v, wsem.at[0])
    c_wq = pltpu.make_async_copy(wqkv_hbm.at[:, 0:512], wqkv_v.at[:, 0:512], wsem.at[1])
    c_wk = pltpu.make_async_copy(wqkv_hbm.at[:, 512:896], wqkv_v.at[:, 512:896], wsem.at[7])
    c_wv = pltpu.make_async_copy(wqkv_hbm.at[:, 896:1344], wqkv_v.at[:, 896:1344], wsem.at[8])
    c_wo = pltpu.make_async_copy(wo_hbm, wo_v.at[0:D], wsem.at[2])
    c_w1 = pltpu.make_async_copy(w1_hbm, w1_v.at[0:D], wsem.at[3])
    c_w2 = pltpu.make_async_copy(w2T_hbm, w2T_v, wsem.at[4])
    c_b1 = pltpu.make_async_copy(b1_hbm, b1_v, wsem.at[5])
    c_b2 = pltpu.make_async_copy(b2_hbm, b2_v, wsem.at[6])

    c_wphi.start()
    c_wq.start()

    e16 = lax.broadcasted_iota(jnp.int32, (16, TS), 0)
    one_rows = jnp.where(e16 == 0, 1.0, 0.0)

    def ln_tile(j):
        for b in range(TS // 128):
            xn = _layernorm_t(x_v[j, :, 128 * b:128 * (b + 1)])
            xn_v[j, 0:D, 128 * b:128 * (b + 1)] = xn.astype(_BF16)

    for j in range(NTILE):
        xn_v[j, D:DE, :] = one_rows.astype(_BF16)

    wflat_v[...] = jnp.zeros(wflat_v.shape, _F32)
    wf2_v[...] = jnp.zeros(wf2_v.shape, _F32)
    kv_v[...] = jnp.zeros(kv_v.shape, _F32)
    c_wphi.wait()
    wf2_v[:, 0:DH] = wphi_v[...].reshape(D, DH).astype(_F32)
    for h in range(H):
        wflat_v[64 + DH * h:64 + DH * (h + 1), :] = wf2_v[pl.ds(h, DH, stride=H), :]
    wfb = wflat_v[...].astype(_BF16)
    rr = lax.broadcasted_iota(jnp.int32, (2 * GR, 128), 0)
    cc = lax.broadcasted_iota(jnp.int32, (2 * GR, 128), 1)
    fr = jnp.where(rr >= GR, rr - GR, rr) >> 1
    rf = jnp.where(cc == fr, 1.0, 0.0).astype(_BF16)
    uq = _dot(rf, wfb[64:576], _NT)
    uk = _dot(rf, wfb[0:512], _NT)

    def amat(u, c, shift, l0, w):
        row = lax.broadcasted_iota(jnp.int32, (2 * GR, w), 0)
        ln = lax.broadcasted_iota(jnp.int32, (2 * GR, w), 1)
        lo = (jnp.where(row >= GR, 2, 0) + (row & 1)) * DH + (112 * c + shift - l0)
        return jnp.where((ln >= lo) & (ln < lo + DH), u[:, l0:l0 + w], 0.0).astype(_BF16)

    q_win = [(0, 128), (0, 256), (128, 256), (256, 256)]
    k_win = [(0, 256), (128, 256), (256, 256), (384, 128)]
    aq = [amat(uq, c, 0, *q_win[c]) for c in range(4)]
    ak = [amat(uk, c, 64, *k_win[c]) for c in range(4)]
    c_wk.start()
    c_wq.wait()
    x_copy(0).start()
    for c in range(4):
        l0, w = q_win[c]
        wT_v[112 * c:112 * (c + 1), :] = _dot(aq[c], wqkv_v[:, l0:l0 + w], _NT).astype(_BF16)
    c_wk.wait()
    c_wv.start()
    for c in range(4):
        l0, w = k_win[c]
        wT_v[D + 112 * c:D + 112 * (c + 1), :] = _dot(
            ak[c], wqkv_v[:, 384 + l0:384 + l0 + w], _NT).astype(_BF16)
    x_copy(0).wait()
    x_copy(1).start()
    ln_tile(0)
    c_wv.wait()
    for i in range(2, NTILE):
        x_copy(i).start()
    wT_v[2 * D:3 * D, :] = wqkv_v[:, 2 * D:3 * D].T
    c_b1.start()
    c_b2.start()
    c_wo.start()
    c_w1.start()
    c_w2.start()

    def phase1(i, carry):
        @pl.when(i + 1 < NTILE)
        def _():
            x_copy(i + 1).wait()
        xn = xn_v[i, 0:D, :]
        vT = _dot(wT_v[2 * D:3 * D, :], xn, _NN)
        ln_tile(jnp.minimum(i + 1, NTILE - 1))
        phik = []
        for c in range(4):
            p = _dot(wT_v[D + 112 * c:D + 112 * (c + 1), :], xn, _NN)
            phik.append(_dual_softmax(p[0:GR]))
            phik.append(_dual_softmax(p[GR:2 * GR]))
        ones = jnp.ones((8, TS), _F32)

        def kv(g):
            vext = jnp.concatenate([vT[GR * g:GR * (g + 1)], ones], axis=0).astype(_BF16)
            kv_v[g] += _dot(vext, phik[g], _NT)

        kv_after = {0: [], 1: [0, 1], 2: [2, 3], 3: [4, 5, 6, 7]}
        for c in range(4):
            p = _dot(wT_v[112 * c:112 * (c + 1), :], xn, _NN)
            phiq_v[i, 224 * c:224 * c + 112, :] = _dual_softmax(p[0:GR])
            phiq_v[i, 224 * c + 112:224 * (c + 1), :] = _dual_softmax(p[GR:2 * GR])
            for g in kv_after[c]:
                kv(g)
        return carry

    lax.fori_loop(0, NTILE, phase1, 0)

    r2 = lax.broadcasted_iota(jnp.int32, (64, 2 * GR), 0)
    c2 = lax.broadcasted_iota(jnp.int32, (64, 2 * GR), 1)
    rhead = jnp.where(r2 < GR, (r2 >= DH).astype(jnp.int32), (r2 >= GR + 4).astype(jnp.int32))
    keep = rhead == (c2 & 1)
    c_b1.wait()
    c_b2.wait()
    c_wo.wait()
    c_w1.wait()
    c_w2.wait()
    for g in range(NG):
        kvm_v[g] = jnp.where(keep, kv_v[g], 0.0).astype(_BF16)
    b1 = b1_v[...].astype(_F32).reshape(1, F)
    b2 = b2_v[...].astype(_F32).reshape(1, D)
    wo_v[D:DE, :] = jnp.where(lax.broadcasted_iota(jnp.int32, (16, D), 0) == 0, b2, 0.0).astype(_BF16)
    w1_v[D:DE, :] = jnp.where(lax.broadcasted_iota(jnp.int32, (16, F), 0) == 0, b1, 0.0).astype(_BF16)
    sub = lax.broadcasted_iota(jnp.int32, (8, TS), 0)

    def phase2(i, carry):
        oT = []
        for g in range(NG):
            n = _dot(kvm_v[g], phiq_v[i, 112 * g:112 * (g + 1), :], _NN)
            r = 1.0 / (n[GR:GR + 8] + 1e-6)
            rs = pltpu.roll(r, 4, axis=0)
            ra = jnp.where(sub < 4, r, rs)
            rb = jnp.where(sub < 4, rs, r)
            oT.append((n[0:24].reshape(3, 8, TS) * ra[None]).reshape(24, TS))
            oT.append(n[24:32] * r)
            oT.append((n[32:56].reshape(3, 8, TS) * rb[None]).reshape(24, TS))
        oT.append(one_rows)
        oT = jnp.concatenate(oT, axis=0).astype(_BF16)
        xnat = xn_v[i].T
        h = _gelu(_dot(xnat, w1_v[...], _NN)).astype(_BF16)
        woT = wo_v[...].T
        acc = _dot(w2T_v[...], h, _NT) + x_v[i].astype(_F32)
        for p in range(NS):
            o = acc[:, HS * p:HS * (p + 1)] + _dot(woT, oT[:, HS * p:HS * (p + 1)], _NN)
            out_v[i, :, HS * p:HS * (p + 1)] = o.astype(_BF16)
            out_copy(i, p).start()
        return carry

    lax.fori_loop(0, NTILE, phase2, 0)
    for i in range(NTILE):
        for p in range(NS):
            out_copy(i, p).wait()


@jax.jit
def pallas_parallel_sum__linear_kernel_hedgehog__dense_activation_gelu__prompt_kernel(
    A_x: jax.Array,
    A_wqkv: jax.Array,
    A_w_phi: jax.Array,
    A_wo: jax.Array,
    B_x: jax.Array,
    B_w1: jax.Array,
    B_b1: jax.Array,
    B_w2: jax.Array,
    B_b2: jax.Array,
):
    del B_x
    hbm_spec = pl.BlockSpec(memory_space=pltpu.HBM)
    scratch = [
        pltpu.VMEM((NTILE, D, TS), _BF16),
        pltpu.VMEM((D, 3 * D), _BF16),
        pltpu.VMEM((DH, H, DH), _BF16),
        pltpu.VMEM((DE, D), _BF16),
        pltpu.VMEM((DE, F), _BF16),
        pltpu.VMEM((F,), _BF16),
        pltpu.VMEM((D, F), _BF16),
        pltpu.VMEM((D,), _BF16),
        pltpu.VMEM((NTILE, D, TS), _BF16),
        pltpu.VMEM((NTILE, DE, TS), _BF16),
        pltpu.VMEM((3 * D, D), _BF16),
        pltpu.VMEM((D, 128), _F32),
        pltpu.VMEM((576, 128), _F32),
        pltpu.VMEM((NTILE, 2 * D, TS), _BF16),
        pltpu.VMEM((NG, 64, 2 * GR), _F32),
        pltpu.VMEM((NG, 64, 2 * GR), _BF16),
        pltpu.SemaphoreType.DMA((NTILE,)),
        pltpu.SemaphoreType.DMA((9,)),
        pltpu.SemaphoreType.DMA((NS * NTILE,)),
    ]
    outT = pl.pallas_call(
        _kernel,
        in_specs=[hbm_spec] * 8,
        out_specs=hbm_spec,
        out_shape=jax.ShapeDtypeStruct((1, D, S), _BF16),
        scratch_shapes=scratch,
        compiler_params=pltpu.CompilerParams(vmem_limit_bytes=100 * 1024 * 1024),
    )(jnp.transpose(A_x, (0, 2, 1)), A_wqkv, jnp.transpose(A_w_phi, (1, 0, 2)), A_wo,
      B_w1, B_b1, B_w2.T, B_b2)
    return jnp.transpose(outT, (0, 2, 1))
```
